```python
import os as _os
_os.environ.setdefault('JAX_PLATFORMS', 'cpu')
import jax
import jax.numpy as jnp

def _softmax(x, axis=-1):
    return jax.nn.softmax(x, axis=axis)

def _gelu(x):
    return jax.nn.gelu(x, approximate=True)

def _silu(x):
    return jax.nn.silu(x)

def _sigmoid(x):
    return jax.nn.sigmoid(x)

def _layernorm(x, axis=-1, eps=1e-05):
    m = jnp.mean(x, axis=axis, keepdims=True)
    v = jnp.var(x, axis=axis, keepdims=True)
    return (x - m) / jnp.sqrt(v + eps)

def _scatter_add(tgt, idx, src, axis=0):
    return tgt.at[idx].add(src)

def _segment_sum(src, seg, n):
    return jax.ops.segment_sum(src, seg, n)

class _Rng:

    def __init__(self, key):
        self._k = key

    def _next(self):
        self._k, sub = jax.random.split(self._k)
        return sub

    def normal(self, shape):
        return jax.random.normal(self._next(), shape, dtype=jnp.bfloat16)

    def randint(self, lo, hi, shape):
        return jax.random.randint(self._next(), shape, lo, hi, dtype=jnp.int32)

    def uniform(self, shape, lo=0.0, hi=1.0):
        return jax.random.uniform(self._next(), shape, jnp.bfloat16, lo, hi)

    def permutation(self, n):
        return jax.random.permutation(self._next(), n)
kernel_name = 'adaLN_cond__mha_block__dense_activation_squared_relu__prompt'

def setup_inputs():
    _rng = _Rng(jax.random.key(int.from_bytes(__import__("os").urandom(4), "little")))
    _w = lambda a: (lambda t: t.astype(jnp.bfloat16) if jnp.issubdtype(t.dtype, jnp.floating) else t)(jnp.asarray(a))

    def _A_setup():
        B, S, D, H = (1, 2048, 512, 32)
        return {'x': _w((lambda *s: _rng.normal(s) * 0.05)(B, S, D)), 'wqkv': _w((lambda *s: _rng.normal(s) * 0.1)(D, 3 * D)), 'wo': _w((lambda *s: _rng.normal(s) * 0.05)(D, D))}
    _A_in = _A_setup()

    def _B_setup():
        B, S, D, F = (1, 2048, 512, 1792)
        return {'x': _w((lambda *s: _rng.normal(s) * 0.05)(B, S, D)), 'w1': _w((lambda *s: _rng.normal(s) * 0.05)(D, F)), 'b1': _w((lambda *s: _rng.normal(s) * 0.05)(F)), 'w2': _w((lambda *s: _rng.normal(s) * 0.05)(F, D)), 'b2': _w((lambda *s: _rng.normal(s) * 0.05)(D))}
    _B_in = _B_setup()
    return {'A_x': _A_in['x'], 'A_wqkv': _A_in['wqkv'], 'A_wo': _A_in['wo'], 'B_x': _B_in['x'], 'B_w1': _B_in['w1'], 'B_b1': _B_in['b1'], 'B_w2': _B_in['w2'], 'B_b2': _B_in['b2'], 'c': _w((lambda *s: _rng.normal(s) * 0.05)(1, 512) * 8.0), 'w_mod': _w((lambda *s: _rng.normal(s) * 0.05)(512, 6 * 512) * 512 ** (-0.5) * 8.0)}

def reference(A_x, A_wqkv, A_wo, B_x, B_w1, B_b1, B_w2, B_b2, c, w_mod):

    def _A_ref(x, wqkv, wo):
        B, S, D = x.shape
        H = 32
        Dh = D // H
        qkv = (lambda x, *d: x.transpose(*d))((x @ wqkv).reshape(B, S, 3, H, Dh), 2, 0, 3, 1, 4)
        q, k, v = (qkv[0], qkv[1], qkv[2])
        scores = jnp.einsum('bhqd,bhkd->bhqk', q, k) * Dh ** (-0.5)
        p = _softmax(scores, axis=-1)
        o = jnp.einsum('bhqk,bhkd->bhqd', p, v)
        return (lambda x, *d: x.transpose(*d))(o, 0, 2, 1, 3).reshape(B, S, D) @ wo

    def _B_ref(x, w1, b1, w2, b2):
        h = jnp.einsum('bsd,df->bsf', x, w1) + b1
        zero = jnp.zeros_like(h)
        r = jnp.where(h > zero, h, zero)
        h = r * r
        out = jnp.einsum('bsf,fd->bsd', h, w2) + b2
        return out
    x = A_x
    mod = (_silu(c) @ w_mod).reshape(c.shape[0], 6, 1, -1)
    sa, ca, ga, sb, cb, gb = (mod[:, 0].copy(), mod[:, 1].copy(), mod[:, 2].copy(), mod[:, 3].copy(), mod[:, 4].copy(), mod[:, 5].copy())
    h = _layernorm(x, axis=-1) * (1 + ca) + sa
    x = x + ga * _A_ref(h, A_wqkv, A_wo)
    h = _layernorm(x, axis=-1) * (1 + cb) + sb
    x = x + gb * _B_ref(h, B_w1, B_b1, B_w2, B_b2)
    return x
```

```python
import functools
import math
import jax
import jax.numpy as jnp
from jax import lax
import jax.experimental.pallas as pl
import jax.experimental.pallas.tpu as pltpu

S = 2048
D = 512
H = 32
DH = 16
F = 1792
EPS = 1e-5
TQ = 512
NQT = S // TQ
KB = 256
NKB = S // KB
NU = H * NQT
RT = 512
QSCALE = (DH ** -0.5) * math.log2(math.e)


def _ln(x):
    mu = jnp.mean(x, axis=-1, keepdims=True)
    xc = x - mu
    var = jnp.mean(xc * xc, axis=-1, keepdims=True)
    return xc * lax.rsqrt(var + EPS)


def _kernel(x_ref, wqkv_ref, wo_ref, w1_ref, b1_ref, w2_ref, b2_ref, c_ref, wmod_ref,
            o_ref,
            mod_ref, qt_ref, k_ref, vt_ref, at_ref, s0_ref, s1_ref, m0_ref, m1_ref):
    f32 = jnp.float32
    bf16 = jnp.bfloat16

    c = c_ref[...].astype(f32)
    sc = c * jax.nn.sigmoid(c)
    mod_ref[...] = jnp.dot(sc.astype(bf16), wmod_ref[...], preferred_element_type=f32)

    sa = mod_ref[:, 0 * D:1 * D]
    ca = mod_ref[:, 1 * D:2 * D]
    for r in range(S // RT):
        rows = pl.ds(r * RT, RT)
        x = x_ref[rows, :].astype(f32)
        h = (_ln(x) * (1.0 + ca) + sa).astype(bf16)
        q = jnp.dot(h, wqkv_ref[:, 0 * D:1 * D], preferred_element_type=f32) * QSCALE
        qt = q.T.astype(bf16)
        for g in range(4):
            for tt in range(RT // TQ):
                qt_ref[g, r * (RT // TQ) + tt] = qt[g * 128:(g + 1) * 128, tt * TQ:(tt + 1) * TQ]
        k = jnp.dot(h, wqkv_ref[:, 1 * D:2 * D], preferred_element_type=f32).astype(bf16)
        for g in range(4):
            k_ref[g, rows, :] = k[:, g * 128:(g + 1) * 128]
        v = jnp.dot(h, wqkv_ref[:, 2 * D:3 * D], preferred_element_type=f32)
        vt_ref[:, rows] = v.T.astype(bf16)

    row_head = lax.broadcasted_iota(jnp.int32, (128, TQ), 0) // DH
    ones_blk = jnp.ones((DH, KB), bf16)

    def step(n_qk, s_cur, m_cur, n_sm, s_prev, m_prev):
        if n_qk is not None:
            hq = n_qk // NQT
            tq = n_qk % NQT
            g = hq // 8
            qtm = jnp.where(row_head == hq % 8, qt_ref[g, tq], jnp.zeros((), bf16))
            m_run = jnp.full((8, TQ), -jnp.inf, f32)
        if n_sm is not None:
            hs = n_sm // NQT
            ts = n_sm % NQT
            mp = m_prev[...]
            acc = jnp.zeros((2 * DH, TQ), f32)
        for kb in range(NKB):
            krows = pl.ds(kb * KB, KB)
            if n_qk is not None:
                s = jnp.dot(k_ref[g, krows, :], qtm, preferred_element_type=f32)
                s_cur[krows, :] = s
                m_run = jnp.maximum(m_run, jnp.max(s.reshape(KB // 8, 8, TQ), axis=0))
            if n_sm is not None:
                p = jnp.exp2(s_prev[krows, :] - mp).astype(bf16)
                vte = jnp.concatenate(
                    [vt_ref[pl.ds(pl.multiple_of(hs * DH, DH), DH), krows], ones_blk], axis=0)
                acc = acc + jnp.dot(vte, p, preferred_element_type=f32)
        if n_qk is not None:
            m_cur[...] = jnp.max(m_run, axis=0, keepdims=True)
        if n_sm is not None:
            o = acc[0:DH] / acc[DH:DH + 1]
            at_ref[hs, ts] = o.astype(bf16)

    step(0, s0_ref, m0_ref, None, None, None)

    def loop_body(i, carry):
        n = 2 * i + 1
        step(n, s1_ref, m1_ref, n - 1, s0_ref, m0_ref)
        step(n + 1, s0_ref, m0_ref, n, s1_ref, m1_ref)
        return carry

    lax.fori_loop(0, (NU - 2) // 2, loop_body, 0)
    step(NU - 1, s1_ref, m1_ref, NU - 2, s0_ref, m0_ref)
    step(None, None, None, NU - 1, s1_ref, m1_ref)

    ga = mod_ref[:, 2 * D:3 * D]
    sb = mod_ref[:, 3 * D:4 * D]
    cb = mod_ref[:, 4 * D:5 * D]
    gb = mod_ref[:, 5 * D:6 * D]
    for t in range(NQT):
        rows = pl.ds(t * TQ, TQ)
        att = at_ref[:, t].reshape(D, TQ)
        a = att.astype(f32).T.astype(bf16)
        y = jnp.dot(a, wo_ref[...], preferred_element_type=f32)
        x1 = x_ref[rows, :].astype(f32) + ga * y
        h2 = (_ln(x1) * (1.0 + cb) + sb).astype(bf16)
        u = jnp.dot(h2, w1_ref[...], preferred_element_type=f32) + b1_ref[...].astype(f32)
        r = jnp.maximum(u, 0.0)
        z = jnp.dot((r * r).astype(bf16), w2_ref[...], preferred_element_type=f32) + b2_ref[...].astype(f32)
        o_ref[rows, :] = (x1 + gb * z).astype(o_ref.dtype)


@jax.jit
def pallas_adaLN_cond__mha_block__dense_activation_squared_relu__prompt_kernel(
        A_x, A_wqkv, A_wo, B_x, B_w1, B_b1, B_w2, B_b2, c, w_mod):
    del B_x
    x = A_x.reshape(S, D)
    out = pl.pallas_call(
        _kernel,
        out_shape=jax.ShapeDtypeStruct((S, D), A_x.dtype),
        scratch_shapes=[
            pltpu.VMEM((1, 6 * D), jnp.float32),
            pltpu.VMEM((4, NQT, 128, TQ), jnp.bfloat16),
            pltpu.VMEM((4, S, 128), jnp.bfloat16),
            pltpu.VMEM((D, S), jnp.bfloat16),
            pltpu.VMEM((H, NQT, DH, TQ), jnp.bfloat16),
            pltpu.VMEM((S, TQ), jnp.float32),
            pltpu.VMEM((S, TQ), jnp.float32),
            pltpu.VMEM((1, TQ), jnp.float32),
            pltpu.VMEM((1, TQ), jnp.float32),
        ],
        compiler_params=pltpu.CompilerParams(vmem_limit_bytes=100 * 2 ** 20),
    )(x, A_wqkv, A_wo, B_w1, B_b1.reshape(1, F), B_w2, B_b2.reshape(1, D), c, w_mod)
    return out.reshape(1, S, D)
```

```python
import math

import jax
import jax.numpy as jnp
from jax import lax
import jax.experimental.pallas as pl
import jax.experimental.pallas.tpu as pltpu

S = 2048
D = 512
H = 32
DH = 16
F = 1792
EPS = 1e-5
TQ = 512
KB = 128
UPB = 4
RT = 512
NQT = S // TQ
NKB = S // KB
NU = H * NQT
NB = NU // UPB
NRT = S // RT
QSCALE = (DH ** -0.5) * math.log2(math.e)


def _ln(x):
    mu = jnp.mean(x, axis=-1, keepdims=True)
    xc = x - mu
    var = jnp.mean(xc * xc, axis=-1, keepdims=True)
    return xc * lax.rsqrt(var + EPS)


def _kernel(x_hbm, wqkv_hbm, wo_hbm, w1_hbm, b1_ref, w2_hbm, b2_ref, c_ref, wmod_hbm,
            o_hbm,
            x_ref, wqkv_ref, wo_ref, w1_ref, w2_ref, wmod_ref, ob_ref,
            mod_ref, qt_ref, k_ref, vt_ref, at_ref, s_ref, m_ref,
            in_sems, out_sems):
    f32 = jnp.float32
    bf16 = jnp.bfloat16

    def x_copy(r):
        rows = pl.ds(pl.multiple_of(r * RT, RT), RT)
        return pltpu.make_async_copy(x_hbm.at[rows], x_ref.at[rows], in_sems.at[r])

    wmod_a = pltpu.make_async_copy(wmod_hbm.at[:, pl.ds(0, 2 * D)], wmod_ref.at[:, pl.ds(0, 2 * D)],
                                   in_sems.at[NRT])
    wqkv_c = pltpu.make_async_copy(wqkv_hbm, wqkv_ref, in_sems.at[NRT + 1])
    wmod_b = pltpu.make_async_copy(wmod_hbm.at[:, pl.ds(2 * D, 4 * D)], wmod_ref.at[:, pl.ds(2 * D, 4 * D)],
                                   in_sems.at[NRT + 2])
    wo_c = pltpu.make_async_copy(wo_hbm, wo_ref, in_sems.at[NRT + 3])
    w1_c = pltpu.make_async_copy(w1_hbm, w1_ref, in_sems.at[NRT + 4])
    w2_c = pltpu.make_async_copy(w2_hbm, w2_ref, in_sems.at[NRT + 5])

    wmod_a.start()
    x_copy(0).start()
    wqkv_c.start()
    for r in range(1, NRT):
        x_copy(r).start()

    c = c_ref[...].astype(f32)
    sc = (c * jax.nn.sigmoid(c)).astype(bf16)
    wmod_a.wait()
    mod_ref[:, 0:2 * D] = jnp.dot(sc, wmod_ref[:, 0:2 * D], preferred_element_type=f32)

    sa = mod_ref[:, 0 * D:1 * D]
    ca = mod_ref[:, 1 * D:2 * D]
    wqkv_c.wait()

    def p1_body(r, carry):
        rows = pl.ds(pl.multiple_of(r * RT, RT), RT)
        x_copy(r).wait()
        x = x_ref[rows, :].astype(f32)
        h = (_ln(x) * (1.0 + ca) + sa).astype(bf16)
        q = jnp.dot(h, wqkv_ref[:, 0 * D:1 * D], preferred_element_type=f32) * QSCALE
        qt = q.T.astype(bf16)
        for g in range(4):
            qt_ref[g, r] = qt[g * 128:(g + 1) * 128, :]
        k = jnp.dot(h, wqkv_ref[:, 1 * D:2 * D], preferred_element_type=f32).astype(bf16)
        for g in range(4):
            k_ref[g, rows, :] = k[:, g * 128:(g + 1) * 128]
        v = jnp.dot(h, wqkv_ref[:, 2 * D:3 * D], preferred_element_type=f32)
        vt_ref[r] = v.T.astype(bf16)
        return carry

    lax.fori_loop(0, NRT, p1_body, 0)
    wmod_b.start()
    wo_c.start()
    w1_c.start()
    w2_c.start()

    row_head = lax.broadcasted_iota(jnp.int32, (128, TQ), 0) // DH

    def step(n_qk, slot_qk, n_sm, slot_sm):
        if n_qk is not None:
            hq = n_qk // NQT
            g = hq // 8
            qtm = jnp.where(row_head == hq % 8, qt_ref[g, n_qk % NQT], jnp.zeros((), bf16))
            m_run = jnp.full((8, TQ), -jnp.inf, f32)
        if n_sm is not None:
            hs = n_sm // NQT
            mp = m_ref[slot_sm]
            l_run = jnp.zeros((8, TQ), f32)
            acc = None
        for kb in range(NKB):
            krows = pl.ds(kb * KB, KB)
            if n_qk is not None:
                s = jnp.dot(k_ref[g, krows, :], qtm, preferred_element_type=f32)
                s_ref[slot_qk, krows, :] = s
                m_run = jnp.maximum(m_run, jnp.max(s.reshape(KB // 8, 8, TQ), axis=0))
            if n_sm is not None:
                pf = jnp.exp2(s_ref[slot_sm, krows, :] - mp)
                l_run = l_run + jnp.sum(pf.reshape(KB // 8, 8, TQ), axis=0)
                vt = vt_ref[kb * KB // RT, pl.ds(pl.multiple_of(hs * DH, DH), DH),
                            pl.ds((kb * KB) % RT, KB)]
                pv = jnp.dot(vt, pf.astype(bf16), preferred_element_type=f32)
                acc = pv if acc is None else acc + pv
        if n_qk is not None:
            m_ref[slot_qk] = jnp.max(m_run, axis=0, keepdims=True)
        if n_sm is not None:
            o = acc / jnp.sum(l_run, axis=0, keepdims=True)
            at_ref[hs, n_sm % NQT] = o.astype(bf16)

    def block(j, setid, do_qk=True, do_sm=True):
        for u in range(UPB):
            step(j * UPB + u if do_qk else None, setid * UPB + u,
                 (j - 1) * UPB + u if do_sm else None, (1 - setid) * UPB + u)

    block(0, 0, do_sm=False)

    def loop_body(i, carry):
        j = 2 * i + 1

        @pl.when(j < NB)
        def _():
            block(j, 1)

        @pl.when(j + 1 < NB)
        def _():
            block(j + 1, 0)
        return carry

    lax.fori_loop(0, NB // 2, loop_body, 0)
    block(NB, NB % 2, do_qk=False)

    wmod_b.wait()
    wo_c.wait()
    w1_c.wait()
    w2_c.wait()
    mod_ref[:, 2 * D:6 * D] = jnp.dot(sc, wmod_ref[:, 2 * D:6 * D], preferred_element_type=f32)
    ga = mod_ref[:, 2 * D:3 * D]
    sb = mod_ref[:, 3 * D:4 * D]
    cb = mod_ref[:, 4 * D:5 * D]
    gb = mod_ref[:, 5 * D:6 * D]

    def out_copy(t):
        rows = pl.ds(pl.multiple_of(t * RT, RT), RT)
        return pltpu.make_async_copy(ob_ref.at[rows], o_hbm.at[rows], out_sems.at[t])

    def p3_body(t, carry):
        rows = pl.ds(pl.multiple_of(t * RT, RT), RT)
        att = at_ref[:, t].reshape(D, RT)
        a = att.astype(f32).T.astype(bf16)
        y = jnp.dot(a, wo_ref[...], preferred_element_type=f32)
        x1 = x_ref[rows, :].astype(f32) + ga * y
        h2 = (_ln(x1) * (1.0 + cb) + sb).astype(bf16)
        u = jnp.dot(h2, w1_ref[...], preferred_element_type=f32) + b1_ref[...].astype(f32)
        r = jnp.maximum(u, 0.0)
        z = jnp.dot((r * r).astype(bf16), w2_ref[...], preferred_element_type=f32) + b2_ref[...].astype(f32)
        ob_ref[rows, :] = (x1 + gb * z).astype(ob_ref.dtype)
        out_copy(t).start()
        return carry

    lax.fori_loop(0, NRT, p3_body, 0)
    for t in range(NRT):
        out_copy(t).wait()


@jax.jit
def pallas_adaLN_cond__mha_block__dense_activation_squared_relu__prompt_kernel(
        A_x: jax.Array,
        A_wqkv: jax.Array,
        A_wo: jax.Array,
        B_x: jax.Array,
        B_w1: jax.Array,
        B_b1: jax.Array,
        B_w2: jax.Array,
        B_b2: jax.Array,
        c: jax.Array,
        w_mod: jax.Array,
):
    del B_x
    x = A_x.reshape(S, D)
    hbm = pl.BlockSpec(memory_space=pl.ANY)
    vmem = pl.BlockSpec(memory_space=pltpu.VMEM)
    out = pl.pallas_call(
        _kernel,
        out_shape=jax.ShapeDtypeStruct((S, D), A_x.dtype),
        in_specs=[hbm, hbm, hbm, hbm, vmem, hbm, vmem, vmem, hbm],
        out_specs=hbm,
        scratch_shapes=[
            pltpu.VMEM((S, D), jnp.bfloat16),
            pltpu.VMEM((D, 3 * D), jnp.bfloat16),
            pltpu.VMEM((D, D), jnp.bfloat16),
            pltpu.VMEM((D, F), jnp.bfloat16),
            pltpu.VMEM((F, D), jnp.bfloat16),
            pltpu.VMEM((D, 6 * D), jnp.bfloat16),
            pltpu.VMEM((S, D), jnp.bfloat16),
            pltpu.VMEM((1, 6 * D), jnp.float32),
            pltpu.VMEM((4, NQT, 128, TQ), jnp.bfloat16),
            pltpu.VMEM((4, S, 128), jnp.bfloat16),
            pltpu.VMEM((NRT, D, RT), jnp.bfloat16),
            pltpu.VMEM((H, NQT, DH, TQ), jnp.bfloat16),
            pltpu.VMEM((2 * UPB, S, TQ), jnp.float32),
            pltpu.VMEM((2 * UPB, 1, TQ), jnp.float32),
            pltpu.SemaphoreType.DMA((NRT + 6,)),
            pltpu.SemaphoreType.DMA((NRT,)),
        ],
        compiler_params=pltpu.CompilerParams(vmem_limit_bytes=100 * 2 ** 20),
    )(x, A_wqkv, A_wo, B_w1, B_b1.reshape(1, F), B_w2, B_b2.reshape(1, D), c, w_mod)
    return out.reshape(1, S, D)
```
